```python
import os as _os
_os.environ.setdefault("JAX_PLATFORMS", "cpu")
import jax
import jax.numpy as jnp

def _softmax(x, axis=-1):
    return jax.nn.softmax(x, axis=axis)
def _gelu(x):
    return jax.nn.gelu(x, approximate=True)
def _silu(x):
    return jax.nn.silu(x)
def _sigmoid(x):
    return jax.nn.sigmoid(x)
def _layernorm(x, axis=-1, eps=1e-5):
    m = jnp.mean(x, axis=axis, keepdims=True)
    v = jnp.var(x, axis=axis, keepdims=True)
    return (x - m) / jnp.sqrt(v + eps)
def _scatter_add(tgt, idx, src, axis=0):
    return tgt.at[idx].add(src)
def _segment_sum(src, seg, n):
    return jax.ops.segment_sum(src, seg, n)
class _Rng:
    def __init__(self, key):
        self._k = key
    def _next(self):
        self._k, sub = jax.random.split(self._k)
        return sub
    def normal(self, shape):
        return jax.random.normal(self._next(), shape, dtype=jnp.bfloat16)
    def randint(self, lo, hi, shape):
        return jax.random.randint(self._next(), shape, lo, hi, dtype=jnp.int32)
    def uniform(self, shape, lo=0.0, hi=1.0):
        return jax.random.uniform(self._next(), shape, jnp.bfloat16, lo, hi)
    def permutation(self, n):
        return jax.random.permutation(self._next(), n)


kernel_name = 'standalone__cross_network_dcn_v2__recsys'

def setup_inputs():
    _rng = _Rng(jax.random.key(int.from_bytes(__import__("os").urandom(4), "little")))
    _w = (lambda a: (lambda t: t.astype(jnp.bfloat16) if jnp.issubdtype(t.dtype, jnp.floating) else t)(jnp.asarray(a)))
    B, F, D, L = 16384, 26, 16, 6
    Din = min(F * D, 512)
    R = max(Din // 4, 2)
    sc = Din ** -0.5
    return {
        "x0": _w((lambda *s: _rng.normal(s) * 0.05)(B, Din)),
        "U":  _w((lambda *s: _rng.normal(s) * 1.6)(L, Din, R) * sc),
        "V":  _w((lambda *s: _rng.normal(s) * 1.6)(L, R, Din) * sc),
        "bs": _w((lambda *s: _rng.normal(s) * 0.05)(L, Din)),
    }

def reference(x0, U, V, bs):
    x = x0
    for l in range(U.shape[0]):
        h = jnp.einsum('rd,bd->br', V[l], x)
        h = jnp.einsum('dr,br->bd', U[l], h)
        x = x0 * (h + bs[l]) + x
    return x
```

```python
import jax
import jax.numpy as jnp
from jax import lax
import jax.experimental.pallas as pl
import jax.experimental.pallas.tpu as pltpu

_F32 = jnp.float32
_BF16 = jnp.bfloat16


def _dot(a, b):
    return lax.dot_general(a, b, (((1,), (0,)), ((), ())), preferred_element_type=_F32)


@jax.jit
def pallas_standalone__cross_network_dcn_v2__recsys_kernel(
    x0: jax.Array,
    U: jax.Array,
    V: jax.Array,
    bs: jax.Array,
):
    B, D = x0.shape
    L, _, R = U.shape
    bt, gw = 2048, 512
    G, nt, RP = bt // gw, gw // 128, R + 8

    def kernel_function(x_ref, u_ref, v_ref, b_ref, o_ref, vf_ref, ua_ref, g_ref, xb_ref):
        @pl.when(pl.program_id(0) == 0)
        def _():
            bT = b_ref[...].astype(_F32).T
            lane = lax.broadcasted_iota(jnp.int32, (D, 128), 1)
            for l in range(L):
                vf_ref[l] = v_ref[l].astype(_F32)
                bcol = jnp.broadcast_to(bT[:, l:l + 1], (D, 128))
                up = jnp.concatenate([u_ref[l].astype(_F32), jnp.zeros((D, 128 - R), _F32)], axis=1)
                up = jnp.where(lane == R, bcol, up)
                if l == 0:
                    up = jnp.where(lane == R + 1, 1.0, up)
                ua_ref[l] = up.astype(_BF16)

        row = lax.broadcasted_iota(jnp.int32, (8, gw), 0)
        ones = jnp.where(row < 2, 1.0, 0.0).astype(_F32)
        hs = [None] * G

        def down(l, g):
            if l == 0:
                xg = x_ref[:, g * gw:(g + 1) * gw]
            else:
                xg = jnp.concatenate([xb_ref[g * nt + j] for j in range(nt)], axis=1)
            h = _dot(vf_ref[l], xg)
            hs[g] = jnp.concatenate([h, ones], axis=0).astype(_BF16)

        def up_(l, g):
            s = _dot(ua_ref[l, :, :RP], hs[g])
            if l > 0:
                s = s + g_ref[:, g * gw:(g + 1) * gw]
            x = x_ref[:, g * gw:(g + 1) * gw].astype(_F32) * s
            if l == L - 1:
                o_ref[:, g * gw:(g + 1) * gw] = x.astype(_BF16)
            else:
                g_ref[:, g * gw:(g + 1) * gw] = s
                xq = x.astype(_BF16)
                for j in range(nt):
                    xb_ref[g * nt + j] = xq[:, j * 128:(j + 1) * 128]

        seq = [(l, g) for l in range(L) for g in range(G)]
        down(*seq[0])
        for i, (l, g) in enumerate(seq):
            if i + 1 < len(seq):
                down(*seq[i + 1])
            up_(l, g)

    out = pl.pallas_call(
        kernel_function,
        grid=(B // bt,),
        in_specs=[
            pl.BlockSpec((D, bt), lambda i: (0, i)),
            pl.BlockSpec((L, D, R), lambda i: (0, 0, 0)),
            pl.BlockSpec((L, R, D), lambda i: (0, 0, 0)),
            pl.BlockSpec((L, D), lambda i: (0, 0)),
        ],
        out_specs=pl.BlockSpec((D, bt), lambda i: (0, i)),
        out_shape=jax.ShapeDtypeStruct((D, B), x0.dtype),
        scratch_shapes=[
            pltpu.VMEM((L, R, D), _F32),
            pltpu.VMEM((L, D, 128), _BF16),
            pltpu.VMEM((D, bt), _F32),
            pltpu.VMEM((bt // 128, D, 128), _BF16),
        ],
        compiler_params=pltpu.CompilerParams(
            dimension_semantics=("arbitrary",), vmem_limit_bytes=100 * 1024 * 1024),
    )(x0.T, U, V, bs)
    return out.T
```

```python
import jax
import jax.numpy as jnp
from jax import lax
import jax.experimental.pallas as pl
import jax.experimental.pallas.tpu as pltpu

_F32, _BF16, _I32 = jnp.float32, jnp.bfloat16, jnp.int32
_DOWN, _UP = 0, 1
_TILE = 128
_GROUP = 256
_PEELED = 7
_PER_STEP = 19
_CLASSES = 4


def _dot(a, b):
    return lax.dot_general(a, b, (((1,), (0,)), ((), ())), preferred_element_type=_F32)


def _skewed(slots):
    ops = [(_DOWN,) + slots[0]]
    for i, slot in enumerate(slots):
        if i + 1 < len(slots):
            ops.append((_DOWN,) + slots[i + 1])
        ops.append((_UP,) + slot)
    return ops


def _step_ops(n, layers):
    stagger = 2
    slots = [(g, l) for l in range(layers - 2) for g in range(n)]
    for i in range(n + stagger):
        if i < n:
            slots.append((i, layers - 2))
        if i >= stagger:
            slots.append((i - stagger, layers - 1))
    last = layers - 1
    end = [(_UP, n - 1, last - 1), (_UP, n - 3, last), (_DOWN, n - 2, last),
           (_DOWN, n - 1, last), (_UP, n - 2, last), (_UP, n - 1, last)]
    return [op for op in _skewed(slots) if op not in end] + end


def _cross_kernel(x_hbm, u_hbm, v_hbm, b_hbm, o_hbm,
                  x_ref, o_ref, u_ref, v_ref, b_ref,
                  vp_ref, vt_ref, vs_ref, vc_ref, ua_ref, g_ref, xl_ref,
                  x_sem, o_sem, w_sem):
    L, D, R = u_ref.shape
    n_groups = x_ref.shape[0]
    n_steps = (n_groups - _PEELED) // _PER_STEP
    full = D // _TILE * _TILE
    rem = D - full
    per = R // 8 // _CLASSES * 8
    left = R - _CLASSES * per
    first = [i * per + (left if i else 0) for i in range(_CLASSES)]
    half = D // 2

    def columns(g):
        start = g * _GROUP
        return pl.ds(start if isinstance(g, int) else pl.multiple_of(start, _GROUP), _GROUP)

    def x_copy(g, sem):
        return pltpu.make_async_copy(x_hbm.at[:, columns(g)], x_ref.at[g], sem)

    def o_copy(g, r0, rows):
        return pltpu.make_async_copy(
            o_ref.at[g, pl.ds(r0, rows)], o_hbm.at[pl.ds(r0, rows), columns(g)], o_sem)

    def weight_copies(l0, l1, sem):
        ls = pl.ds(l0, l1 - l0)
        return [pltpu.make_async_copy(v_hbm.at[ls], v_ref.at[ls], sem),
                pltpu.make_async_copy(u_hbm.at[ls], u_ref.at[ls], sem)]

    def prepare_v(l):
        v = v_ref[l].astype(_F32)
        vp_ref[l] = v[:, _TILE:full]
        w = v[:, :_TILE]
        e = jnp.concatenate([v[:, full:], jnp.zeros((R, _TILE - rem), _F32)], axis=1)
        block = lax.broadcasted_iota(_I32, (per, _TILE), 1) // rem
        shared = jnp.zeros((per, _TILE), _F32)
        for i, r in enumerate(first):
            shared = jnp.where(block == i, w[r:r + per], shared)
        vs_ref[l] = shared
        for i, r in enumerate(first):
            e_i = pltpu.roll(e[r:r + per], i * rem, 1) if i else e[r:r + per]
            vt_ref[l, r:r + per] = jnp.where(block == i, e_i, w[r:r + per] - shared)
        lane = lax.broadcasted_iota(_I32, (8, _TILE), 1)
        sub = lax.broadcasted_iota(_I32, (8, _TILE), 0)
        w_left = w[per:per + left]
        vt_ref[l, per:per + left] = jnp.where(lane < rem, e[per:per + left], w_left)
        for s in range(8):
            w_s = pltpu.roll(w_left, s, 0) if s else w_left
            for j in range(rem // 8):
                c = jnp.sum(jnp.where(lane == sub + 8 * j, w_s, 0.0), axis=1, keepdims=True)
                vc_ref[l, s * (rem // 8) + j] = jnp.broadcast_to(c, (8, _TILE))

    def bias_columns():
        rows = jnp.concatenate(
            [jnp.zeros((R, D), _F32), b_ref[...].astype(_F32), jnp.ones((1, D), _F32),
             jnp.zeros((_TILE - R - L - 1, D), _F32)], axis=0)
        return rows.T

    def prepare_u(l, bias):
        ua_ref[l] = jnp.concatenate([u_ref[l].astype(_F32), bias[:, R:]], axis=1)

    row = lax.broadcasted_iota(_I32, (8, _GROUP), 0)
    hidden = {}

    def down(g0, slot, g, l):
        x = x_ref[g0 + g] if l == 0 else xl_ref[slot, g]
        plain = _dot(vp_ref[l], x[_TILE:full])
        own = []
        for i, r in enumerate(first):
            pieces = [x[:i * rem]] if i else []
            pieces.append(x[full:])
            if (i + 1) * rem < _TILE:
                pieces.append(x[(i + 1) * rem:_TILE])
            rows = per if i else per + left
            own.append(_dot(vt_ref[l, r:r + rows], jnp.concatenate(pieces, axis=0)))
        shared = _dot(vs_ref[l], x[:_TILE])
        xf = x[:rem].astype(_F32)
        acc = None
        for s in range(7, -1, -1):
            if acc is not None:
                acc = pltpu.roll(acc, 7, 0)
            for j in range(rem // 8):
                c = vc_ref[l, s * (rem // 8) + j]
                term = jnp.concatenate([c] * (_GROUP // _TILE), axis=1) * xf[8 * j:8 * j + 8]
                acc = term if acc is None else acc + term
        parts = []
        for i, r in enumerate(first):
            parts.append(plain[r:r + per] + own[i][:per] + shared)
            if i == 0:
                parts.append(plain[per:per + left] + own[0][per:] + acc)
        pick = (row == l) | (row == L) if l == 0 else (row == l)
        parts.append(jnp.where(pick, 1.0, 0.0).astype(_F32))
        hidden[g] = jnp.concatenate(parts, axis=0).astype(_BF16)

    def up(g0, slot, g, l, chunks=None):
        h = hidden.pop(g)
        y = jnp.concatenate(
            [_dot(ua_ref[l, r:r + half, :R + 8], h) for r in (0, half)], axis=0)
        for r, rows in chunks or [(0, D)]:
            rs = pl.ds(r, rows)
            gate = y[r:r + rows]
            if l > 0:
                gate = gate + g_ref[slot, g, rs]
            x = (x_ref[g0 + g, rs].astype(_F32) * gate).astype(_BF16)
            if l < L - 1:
                g_ref[slot, g, rs] = gate
                xl_ref[slot, g, rs] = x
            else:
                o_ref[g0 + g, rs] = x
                o_copy(g0 + g, r, rows).start()

    def by_layer(groups, layers):
        return [(op, g, l) for l in layers for op in (_DOWN, _UP) for g in groups]

    mid = L // 2
    phases = [
        (weight_copies(0, 1, w_sem.at[0])
         + [pltpu.make_async_copy(b_hbm, b_ref, w_sem.at[0]),
            x_copy(0, w_sem.at[0]), x_copy(1, w_sem.at[0])],
         range(1), by_layer((0, 1), range(1))),
        (weight_copies(1, mid, w_sem.at[1]), range(1, mid), by_layer((0, 1), range(1, mid))),
        (weight_copies(mid, L, w_sem.at[2]), range(mid, L), by_layer((0, 1), range(mid, L))),
        ([x_copy(g, w_sem.at[3]) for g in range(2, _PEELED)], (),
         _skewed([(g, l) for l in range(L) for g in range(2, _PEELED)])),
    ]
    for copies, _, _ in phases[:3]:
        for copy in copies:
            copy.start()
    fetch_at = [int(_PEELED * L * (0.15 + 0.55 * k / _PER_STEP)) for k in range(_PER_STEP)]
    done = 0
    for i, (copies, layers, ops) in enumerate(phases):
        for copy in copies:
            copy.wait()
        if i == 0:
            bias = bias_columns()
            for copy in phases[3][0]:
                copy.start()
        for l in layers:
            prepare_v(l)
            prepare_u(l, bias)
        for op, g, l in ops:
            if op == _DOWN:
                down(0, 0, g, l)
            else:
                up(0, 0, g, l)
                for k in range(_PER_STEP):
                    if fetch_at[k] == done:
                        x_copy(_PEELED + k, x_sem.at[0]).start()
                done += 1

    head = 64
    last_chunks = [(0, head), (half, head), (head, half - head), (half + head, half - head)]

    def step(it, carry):
        g0 = _PEELED + it * _PER_STEP
        slot = it % 2
        for g in range(_PER_STEP):
            x_copy(g0 + g, x_sem.at[slot]).wait()
        for op, g, l in _step_ops(_PER_STEP, L):
            if op == _DOWN:
                down(g0, slot, g, l)
                continue
            up(g0, slot, g, l, last_chunks if l == L - 1 and g >= _PER_STEP - 2 else None)
            if l == 1:
                @pl.when(it + 1 < n_steps)
                def _():
                    x_copy(g0 + _PER_STEP + g, x_sem.at[1 - slot]).start()
        return carry

    lax.fori_loop(0, n_steps, step, 0)
    pltpu.make_async_copy(o_ref, o_ref, o_sem).wait()


@jax.jit
def pallas_standalone__cross_network_dcn_v2__recsys_kernel(
    x0: jax.Array,
    U: jax.Array,
    V: jax.Array,
    bs: jax.Array,
):
    B, D = x0.shape
    L, _, R = U.shape
    n_groups = B // _GROUP
    per = R // 8 // _CLASSES * 8
    assert B % _GROUP == 0 and (n_groups - _PEELED) % _PER_STEP == 0
    assert D % _TILE * _CLASSES == _TILE and R - _CLASSES * per == 8
    assert 4 <= L < 8 and R + 8 <= _TILE

    hbm = pl.BlockSpec(memory_space=pl.ANY)
    out = pl.pallas_call(
        _cross_kernel,
        in_specs=[hbm] * 4,
        out_specs=hbm,
        out_shape=jax.ShapeDtypeStruct((D, B), x0.dtype),
        scratch_shapes=[
            pltpu.VMEM((n_groups, D, _GROUP), _BF16),
            pltpu.VMEM((n_groups, D, _GROUP), _BF16),
            pltpu.VMEM((L, D, R), _BF16),
            pltpu.VMEM((L, R, D), _BF16),
            pltpu.VMEM((L, D), _BF16),
            pltpu.VMEM((L, R, D // _TILE * _TILE - _TILE), _F32),
            pltpu.VMEM((L, R, _TILE), _F32),
            pltpu.VMEM((L, per, _TILE), _F32),
            pltpu.VMEM((L, D % _TILE, 8, _TILE), _F32),
            pltpu.VMEM((L, D, _TILE), _F32),
            pltpu.VMEM((2, _PER_STEP, D, _GROUP), _F32),
            pltpu.VMEM((2, _PER_STEP, D, _GROUP), _BF16),
            pltpu.SemaphoreType.DMA((2,)),
            pltpu.SemaphoreType.DMA(()),
            pltpu.SemaphoreType.DMA((4,)),
        ],
        compiler_params=pltpu.CompilerParams(
            vmem_limit_bytes=100 * 1024 * 1024,
            disable_bounds_checks=True,
            disable_semaphore_checks=True,
        ),
    )(x0.T, U, V, bs)
    return out.T
```

```python
import jax
import jax.numpy as jnp
from jax import lax
import jax.experimental.pallas as pl
import jax.experimental.pallas.tpu as pltpu

_F32, _BF16, _I32 = jnp.float32, jnp.bfloat16, jnp.int32
_DOWN, _UP = 0, 1
_TILE = 128
_GROUP = 256
_PEELED = 7
_PER_STEP = 19
_CLASSES = 4
_LEFT_CLASS = 1
_PASSES = (
    [("shared", 0)] + [("strassen", k) for k in (5, 0, 4, 1, 3, 2, 6)] + [("shared", 1)]
    + [(i, t) for i in (0, 3, 1, 2) for t in (0, 1)]
)


def _dot(a, b):
    return lax.dot_general(a, b, (((1,), (0,)), ((), ())), preferred_element_type=_F32)


def _skewed(slots):
    ops = [(_DOWN,) + slots[0]]
    for i, slot in enumerate(slots):
        if i + 1 < len(slots):
            ops.append((_DOWN,) + slots[i + 1])
        ops.append((_UP,) + slot)
    return ops


def _step_ops(n, layers):
    stagger = 2
    slots = [(g, l) for l in range(layers - 2) for g in range(n)]
    for i in range(n + stagger):
        if i < n:
            slots.append((i, layers - 2))
        if i >= stagger:
            slots.append((i - stagger, layers - 1))
    last = layers - 1
    end = [(_UP, n - 1, last - 1), (_UP, n - 3, last), (_DOWN, n - 2, last),
           (_DOWN, n - 1, last), (_UP, n - 2, last), (_UP, n - 1, last)]
    return [op for op in _skewed(slots) if op not in end] + end


def _cross_kernel(x_hbm, u_hbm, v_hbm, b_hbm, o_hbm,
                  x_ref, o_ref, u_ref, v_ref, b_ref,
                  v0_ref, vp_ref, vt_ref, vs_ref, vc_ref, ua_ref,
                  g_ref, xp_ref, xq_ref, xr_ref,
                  x_sem, o_sem, w_sem):
    L, D, R = u_ref.shape
    n_groups = x_ref.shape[0]
    n_steps = (n_groups - _PEELED) // _PER_STEP
    half = D // 2
    rem = D % _TILE
    per = R // 8 // _CLASSES * 8
    left = R - _CLASSES * per
    first = [left + i * per for i in range(_CLASSES)]
    top, bottom = slice(left, left + 2 * per), slice(left + 2 * per, R)

    def columns(g):
        start = g * _GROUP
        return pl.ds(start if isinstance(g, int) else pl.multiple_of(start, _GROUP), _GROUP)

    def x_copy(g, sem):
        return pltpu.make_async_copy(x_hbm.at[:, columns(g)], x_ref.at[g], sem)

    def o_copy(g, r0, rows):
        return pltpu.make_async_copy(
            o_ref.at[g, pl.ds(r0, rows)], o_hbm.at[pl.ds(r0, rows), columns(g)], o_sem)

    def weight_copies(l0, l1, sem):
        ls = pl.ds(l0, l1 - l0)
        return [pltpu.make_async_copy(v_hbm.at[ls], v_ref.at[ls], sem),
                pltpu.make_async_copy(u_hbm.at[ls], u_ref.at[ls], sem)]

    def prepare_v(l):
        v = v_ref[l].astype(_F32)
        a1, a2 = v[:, :_TILE], v[:, half:half + _TILE]
        if l == 0:
            v0_ref[...] = jnp.concatenate([a1, a2], axis=1)
        else:
            both = a1[:left] + a2[:left]
            vp_ref[l, 0, :2 * per] = a1[top] + a2[bottom]
            vp_ref[l, 1] = jnp.concatenate([a1[bottom] + a2[bottom], both], axis=0)
            vp_ref[l, 2] = jnp.concatenate([a1[top], a1[:left]], axis=0)
            vp_ref[l, 3] = jnp.concatenate([a2[bottom], a2[:left]], axis=0)
            vp_ref[l, 4] = jnp.concatenate([a1[top] + a2[top], both], axis=0)
            vp_ref[l, 5, :2 * per] = a1[bottom] - a1[top]
            vp_ref[l, 6, :2 * per] = a2[top] - a2[bottom]
        rest = jnp.concatenate(
            [v[:, _TILE:half], v[:, half + _TILE:], jnp.zeros((R, _TILE - rem), _F32)], axis=1)
        w, e = rest[:, :_TILE], rest[:, _TILE:]
        block = lax.broadcasted_iota(_I32, (per, _TILE), 1) // rem
        shared = jnp.zeros((per, _TILE), _F32)
        for i, r in enumerate(first):
            shared = jnp.where(block == i, w[r:r + per], shared)
        vs_ref[l] = shared
        for i, r in enumerate(first):
            e_i = pltpu.roll(e[r:r + per], i * rem, 1) if i else e[r:r + per]
            vt_ref[l, i, :per] = jnp.where(block == i, e_i, w[r:r + per] - shared)
        lane = lax.broadcasted_iota(_I32, (8, _TILE), 1)
        sub = lax.broadcasted_iota(_I32, (8, _TILE), 0)
        w_left = w[:left]
        vt_ref[l, _LEFT_CLASS, per:] = jnp.where(
            lane // rem == _LEFT_CLASS, pltpu.roll(e[:left], _LEFT_CLASS * rem, 1), w_left)
        for s in range(8):
            w_s = pltpu.roll(w_left, s, 0) if s else w_left
            for j in range(rem // 8):
                hit = lane == sub + (_LEFT_CLASS * rem + 8 * j)
                c = jnp.sum(jnp.where(hit, w_s, 0.0), axis=1, keepdims=True)
                vc_ref[l, s * (rem // 8) + j] = jnp.broadcast_to(c, (8, _TILE))

    def bias_columns():
        rows = jnp.concatenate(
            [jnp.zeros((R, D), _F32), b_ref[...].astype(_F32), jnp.ones((1, D), _F32),
             jnp.zeros((_TILE - R - L - 1, D), _F32)], axis=0)
        return pltpu.bitcast(rows.T.astype(_BF16), _I32)

    def prepare_u(l, bias):
        ua_ref[l] = jnp.concatenate([pltpu.bitcast(u_ref[l], _I32), bias[:, R:]], axis=1)

    row = lax.broadcasted_iota(_I32, (8, _GROUP), 0)
    hidden = {}

    def other_rows(x):
        return jnp.concatenate([x[_TILE:half], x[half + _TILE:]], axis=0)

    def left_block(l, x):
        acc = None
        for s in range(7, -1, -1):
            y = None
            for j in range(rem // 8):
                c = vc_ref[l, s * (rem // 8) + j]
                term = jnp.concatenate([c] * (_GROUP // _TILE), axis=1) * x[8 * j:8 * j + 8]
                y = term if y is None else y + term
            acc = y if acc is None else pltpu.roll(acc, 7, 0) + y
        return acc

    def down(g0, slot, g, l):
        if l == 0:
            x = x_ref[g0 + g]
            xr = other_rows(x)
            plain = _dot(v0_ref[...],
                         jnp.concatenate([x[:_TILE], x[half:half + _TILE]], axis=0))
        else:
            xp = xp_ref[slot, g]
            sums = [xp[:, k * _TILE:(k + 1) * _TILE] for k in range(6)]
            xq = xq_ref[slot, g]
            sums.append(jnp.concatenate([xq[:, :_TILE], xq[:, _TILE:]], axis=0))
            xr = xr_ref[slot, g]
        out = {}
        for kind, k in _PASSES:
            if kind == "strassen":
                if l > 0:
                    a = vp_ref[l, k, :2 * per] if k in (0, 5, 6) else vp_ref[l, k]
                    out[kind, k] = _dot(a, sums[k])
                continue
            tile = slice(k * _TILE, (k + 1) * _TILE)
            if kind == "shared":
                out[kind, k] = _dot(vs_ref[l], xr[:_TILE, tile])
            else:
                pieces = [xr[:kind * rem, tile]] if kind else []
                pieces.append(xr[_TILE:, tile])
                if (kind + 1) * rem < _TILE:
                    pieces.append(xr[(kind + 1) * rem:_TILE, tile])
                a = vt_ref[l, kind] if kind == _LEFT_CLASS else vt_ref[l, kind, :per]
                out[kind, k] = _dot(a, jnp.concatenate(pieces, axis=0))
        shared = jnp.concatenate([out["shared", 0], out["shared", 1]], axis=1)
        own = [jnp.concatenate([out[i, 0], out[i, 1]], axis=1) for i in range(_CLASSES)]
        missing = left_block(l, xr[_LEFT_CLASS * rem:(_LEFT_CLASS + 1) * rem].astype(_F32))
        if l > 0:
            m = [out["strassen", k] for k in range(7)]
            n = 2 * per
            plain = jnp.concatenate([
                jnp.concatenate([m[1][n:] + m[3][n:],
                                 (m[3][:n] - m[4][:n]) + m[0] + m[6],
                                 m[1][:n] + m[3][:n]], axis=0),
                jnp.concatenate([m[2][n:] + m[4][n:],
                                 m[2][:n] + m[4][:n],
                                 (m[2][:n] - m[1][:n]) + m[0] + m[5]], axis=0)], axis=1)
        parts = [plain[:left] + own[_LEFT_CLASS][per:] + missing]
        for i, r in enumerate(first):
            parts.append(plain[r:r + per] + own[i][:per] + shared)
        pick = (row == l) | (row == L) if l == 0 else (row == l)
        parts.append(jnp.where(pick, 1.0, 0.0).astype(_F32))
        hidden[g] = jnp.concatenate(parts, axis=0).astype(_BF16)

    def up(g0, slot, g, l, chunks=None):
        h = hidden.pop(g)
        ua = pltpu.bitcast(ua_ref[l], _BF16)
        y = jnp.concatenate([_dot(ua[r:r + half, :R + 8], h) for r in (0, half)], axis=0)
        if l < L - 1:
            gate = y + g_ref[slot, g] if l > 0 else y
            g_ref[slot, g] = gate
            x = x_ref[g0 + g].astype(_F32) * gate
            b11, b12 = x[:_TILE, :_TILE], x[:_TILE, _TILE:]
            b21, b22 = x[half:half + _TILE, :_TILE], x[half:half + _TILE, _TILE:]
            sums = [b11 + b22, b11, b12 - b22, b21 - b11, b22, b11 + b12, b21 + b22]
            xp_ref[slot, g] = jnp.concatenate(sums[:6], axis=1).astype(_BF16)
            xq_ref[slot, g] = jnp.concatenate(
                [sums[6][:_TILE // 2], sums[6][_TILE // 2:]], axis=1).astype(_BF16)
            xr_ref[slot, g] = other_rows(x).astype(_BF16)
            return
        for r, rows in chunks or [(0, D)]:
            rs = pl.ds(r, rows)
            gate = y[r:r + rows] + g_ref[slot, g, rs]
            o_ref[g0 + g, rs] = (x_ref[g0 + g, rs].astype(_F32) * gate).astype(_BF16)
            o_copy(g0 + g, r, rows).start()

    def by_layer(groups, layers):
        return [(op, g, l) for l in layers for op in (_DOWN, _UP) for g in groups]

    mid = L // 2
    phases = [
        (weight_copies(0, 1, w_sem.at[0])
         + [pltpu.make_async_copy(b_hbm, b_ref, w_sem.at[0]),
            x_copy(0, w_sem.at[0]), x_copy(1, w_sem.at[0])],
         range(1), by_layer((0, 1), range(1))),
        (weight_copies(1, mid, w_sem.at[1]), range(1, mid), by_layer((0, 1), range(1, mid))),
        (weight_copies(mid, L, w_sem.at[2]), range(mid, L), by_layer((0, 1), range(mid, L))),
        ([x_copy(g, w_sem.at[3]) for g in range(2, _PEELED)], (),
         _skewed([(g, l) for l in range(L) for g in range(2, _PEELED)])),
    ]
    for copies, _, _ in phases[:3]:
        for copy in copies:
            copy.start()
    fetch_at = [int(_PEELED * L * (0.15 + 0.55 * k / _PER_STEP)) for k in range(_PER_STEP)]
    done = 0
    for i, (copies, layers, ops) in enumerate(phases):
        for copy in copies:
            copy.wait()
        if i == 0:
            bias = bias_columns()
            for copy in phases[3][0]:
                copy.start()
        for l in layers:
            prepare_v(l)
            prepare_u(l, bias)
        for op, g, l in ops:
            if op == _DOWN:
                down(0, 0, g, l)
            else:
                up(0, 0, g, l)
                for k in range(_PER_STEP):
                    if fetch_at[k] == done:
                        x_copy(_PEELED + k, x_sem.at[0]).start()
                done += 1

    head = 64
    last_chunks = [(0, head), (half, head), (head, half - head), (half + head, half - head)]

    def step(it, carry):
        g0 = _PEELED + it * _PER_STEP
        slot = it % 2
        for g in range(_PER_STEP):
            x_copy(g0 + g, x_sem.at[slot]).wait()
        for op, g, l in _step_ops(_PER_STEP, L):
            if op == _DOWN:
                down(g0, slot, g, l)
                continue
            up(g0, slot, g, l, last_chunks if l == L - 1 and g >= _PER_STEP - 2 else None)
            if l == 1:
                @pl.when(it + 1 < n_steps)
                def _():
                    x_copy(g0 + _PER_STEP + g, x_sem.at[1 - slot]).start()
        return carry

    lax.fori_loop(0, n_steps, step, 0)
    pltpu.make_async_copy(o_hbm, o_hbm, o_sem).wait()


@jax.jit
def pallas_standalone__cross_network_dcn_v2__recsys_kernel(
    x0: jax.Array,
    U: jax.Array,
    V: jax.Array,
    bs: jax.Array,
):
    B, D = x0.shape
    L, _, R = U.shape
    n_groups = B // _GROUP
    per = R // 8 // _CLASSES * 8
    assert B % _GROUP == 0 and (n_groups - _PEELED) % _PER_STEP == 0
    assert D // _TILE == 3 and D % _TILE * _CLASSES == _TILE and R - _CLASSES * per == 8
    assert 4 <= L < 8 and R + 8 <= _TILE

    hbm = pl.BlockSpec(memory_space=pl.ANY)
    out = pl.pallas_call(
        _cross_kernel,
        in_specs=[hbm] * 4,
        out_specs=hbm,
        out_shape=jax.ShapeDtypeStruct((D, B), x0.dtype),
        scratch_shapes=[
            pltpu.VMEM((n_groups, D, _GROUP), _BF16),
            pltpu.VMEM((n_groups, D, _GROUP), _BF16),
            pltpu.VMEM((L, D, R), _BF16),
            pltpu.VMEM((L, R, D), _BF16),
            pltpu.VMEM((L, D), _BF16),
            pltpu.VMEM((R, 2 * _TILE), _F32),
            pltpu.VMEM((L, 7, R - 2 * per, _TILE), _F32),
            pltpu.VMEM((L, _CLASSES, per + 8, _TILE), _F32),
            pltpu.VMEM((L, per, _TILE), _F32),
            pltpu.VMEM((L, D % _TILE, 8, _TILE), _F32),
            pltpu.VMEM((L, D // 2, _TILE), _I32),
            pltpu.VMEM((2, _PER_STEP, D, _GROUP), _F32),
            pltpu.VMEM((2, _PER_STEP, _TILE, 6 * _TILE), _BF16),
            pltpu.VMEM((2, _PER_STEP, _TILE // 2, _GROUP), _BF16),
            pltpu.VMEM((2, _PER_STEP, D - 2 * _TILE, _GROUP), _BF16),
            pltpu.SemaphoreType.DMA((2,)),
            pltpu.SemaphoreType.DMA(()),
            pltpu.SemaphoreType.DMA((4,)),
        ],
        compiler_params=pltpu.CompilerParams(
            vmem_limit_bytes=110 * 1024 * 1024,
            disable_bounds_checks=True,
            disable_semaphore_checks=True,
        ),
    )(x0.T, U, V, bs)
    return out.T
```
